```python
import jax
import jax.numpy as jnp

def _softmax(x, axis=-1):
    return jax.nn.softmax(x, axis=axis)
def _gelu(x):
    return jax.nn.gelu(x, approximate=True)
def _silu(x):
    return jax.nn.silu(x)
def _sigmoid(x):
    return jax.nn.sigmoid(x)
def _layernorm(x, axis=-1, eps=1e-5):
    m = jnp.mean(x, axis=axis, keepdims=True)
    v = jnp.var(x, axis=axis, keepdims=True)
    return (x - m) / jnp.sqrt(v + eps)
def _scatter_add(tgt, idx, src, axis=0):
    return tgt.at[idx].add(src)
def _segment_sum(src, seg, n):
    return jax.ops.segment_sum(src, seg, n)
class _Rng:
    def __init__(self, key):
        self._k = key
    def _next(self):
        self._k, sub = jax.random.split(self._k)
        return sub
    def normal(self, shape):
        return jax.random.normal(self._next(), shape, dtype=jnp.bfloat16)
    def randint(self, lo, hi, shape):
        return jax.random.randint(self._next(), shape, lo, hi, dtype=jnp.int32)
    def uniform(self, shape, lo=0.0, hi=1.0):
        return jax.random.uniform(self._next(), shape, jnp.bfloat16, lo, hi)
    def permutation(self, n):
        return jax.random.permutation(self._next(), n)


kernel_name = 'recurrent_scan__sliding_block_cached__mixer_s_mlp__decode'

def setup_inputs():
    _rng = _Rng(jax.random.key(int.from_bytes(__import__("os").urandom(4), "little")))
    _w = (lambda a: (lambda t: t.astype(jnp.bfloat16) if jnp.issubdtype(t.dtype, jnp.floating) else t)(jnp.asarray(a)))
    def _A_setup():
        B, Sq, D = 1, 1, 512
        Hq, Hkv, Sk, Dh = 32, 32, 32768, 128
        assert Hq % Hkv == 0, (Hq, Hkv)
        return {
            "x": _w((lambda *s: _rng.normal(s) * 0.05)(B, Sq, D)),
            "k_cache": _w((lambda *s: _rng.normal(s) * 0.05)(B, Hkv, Sk, Dh)),
            "v_cache": _w((lambda *s: _rng.normal(s) * 0.05)(B, Hkv, Sk, Dh)),
            "wq": _w((lambda *s: _rng.normal(s) * 0.05)(D, Hq * Dh) * (D ** -0.5)),
            "wo": _w((lambda *s: _rng.normal(s) * 0.05)(Hq * Dh, D) * ((Hq * Dh) ** -0.5)),
        }
    _A_in = _A_setup()

    def _B_setup():
        B, S, D, F = 1, 1, 512, 1376
        return {
            "x":  _w((lambda *s: _rng.normal(s) * 0.05)(B, S, D)),
            "w1": _w((lambda *s: _rng.normal(s) * 0.05)(D, D) * (D ** -0.5)),
            "w2": _w((lambda *s: _rng.normal(s) * 0.05)(D, D) * (D ** -0.5)),
            "w3": _w((lambda *s: _rng.normal(s) * 0.05)(D, F) * (D ** -0.5)),
            "w4": _w((lambda *s: _rng.normal(s) * 0.05)(F, D) * (F ** -0.5)),
        }
    _B_in = _B_setup()

    return {
        "A_x": _A_in["x"],
        "A_k_cache": _A_in["k_cache"],
        "A_v_cache": _A_in["v_cache"],
        "A_wq": _A_in["wq"],
        "A_wo": _A_in["wo"],
        "B_x": _B_in["x"],
        "B_w1": _B_in["w1"],
        "B_w2": _B_in["w2"],
        "B_w3": _B_in["w3"],
        "B_w4": _B_in["w4"],
    }

def reference(A_x, A_k_cache, A_v_cache, A_wq, A_wo, B_x, B_w1, B_w2, B_w3, B_w4):
    def _A_ref(x, k_cache, v_cache, wq, wo):
        B, Sq, D = x.shape
        Hq, Dh = 32, 128
        Hkv, Sk = k_cache.shape[1], k_cache.shape[2]
        W = min(4096, max(256, Sk // 4))
        rep = Hq // Hkv
        q = (lambda x, *d: x.transpose(*d))((x @ wq).reshape(B, Sq, Hq, Dh), 0, 2, 1, 3)
        k = jnp.repeat(k_cache[:, :, Sk - W:, :], rep, axis=1)
        v = jnp.repeat(v_cache[:, :, Sk - W:, :], rep, axis=1)
        scores = jnp.einsum("bhqd,bhkd->bhqk", q, k) * (Dh ** -0.5)
        p = _softmax(scores, axis=-1)
        o = jnp.einsum("bhqk,bhkd->bhqd", p, v)
        return (lambda x, *d: x.transpose(*d))(o, 0, 2, 1, 3).reshape(B, Sq, Hq * Dh) @ wo

    def _B_ref(x, w1, w2, w3, w4):
        B, S, D = x.shape
        h = _gelu(_layernorm(x, axis=-1) @ w1)
        c = D // 4
        g0 = jnp.pad(h[:, :, 0*c:1*c], ((0, 0), (1, 0), (0, 0)))[:, :S, :]
        g1 = jnp.pad(h[:, :, 1*c:2*c], ((0, 0), (0, 1), (0, 0)))[:, 1:, :]
        g2 = jnp.pad(h[:, :, 2*c:3*c], ((0, 0), (2, 0), (0, 0)))[:, :S, :]
        g3 = jnp.pad(h[:, :, 3*c:   ], ((0, 0), (0, 2), (0, 0)))[:, 2:, :]
        hs = jnp.concatenate([g0, g1, g2, g3], axis=-1) @ w2
        x1 = x + hs
        h2 = _gelu(_layernorm(x1, axis=-1) @ w3) @ w4
        return x1 + h2

    x = A_x
    xn = _layernorm(x, axis=-1)
    s = _A_ref(xn, A_k_cache, A_v_cache, A_wq, A_wo)
    g = _silu(_B_ref(xn, B_w1, B_w2, B_w3, B_w4))
    return x + s * g
```

```python
import jax
import jax.numpy as jnp
import jax.experimental.pallas as pl
import jax.experimental.pallas.tpu as pltpu

f32, bf16 = jnp.float32, jnp.bfloat16


def _ln(x, eps=1e-5):
    m = jnp.mean(x, axis=-1, keepdims=True)
    xc = x - m
    v = jnp.mean(xc * xc, axis=-1, keepdims=True)
    return xc * jax.lax.rsqrt(v + eps)


def _spans(r0, r1, c):
    out = []
    r = r0
    while r < r1:
        n = min(c, r1 - r)
        out.append((r, n))
        r += n
    return out


def _rr(*ls):
    out = []
    for i in range(max(len(l) for l in ls)):
        for l in ls:
            if i < len(l):
                out.append(l[i])
    return out


@jax.jit
def pallas_recurrent_scan__sliding_block_cached__mixer_s_mlp__decode_kernel(
    A_x: jax.Array,
    A_k_cache: jax.Array,
    A_v_cache: jax.Array,
    A_wq: jax.Array,
    A_wo: jax.Array,
    B_x: jax.Array,
    B_w1: jax.Array,
    B_w2: jax.Array,
    B_w3: jax.Array,
    B_w4: jax.Array,
):
    _, _, D = A_x.shape
    _, H, SK, DH = A_k_cache.shape
    F = B_w3.shape[1]
    W = min(4096, max(256, SK // 4))
    HPG = 2
    NG = H // HPG
    LOOK = 2
    C = 128
    hw = W // 2

    def ch(which, hoff, r0, r1):
        return [(which, hoff, r, n) for r, n in _spans(r0, r1, C)]

    t0 = _rr(ch(0, 0, 0, hw), ch(1, 0, 0, hw), ch(0, 1, 0, hw), ch(1, 1, 0, hw))
    t1 = _rr(ch(0, 0, hw, W), ch(1, 0, hw, W), ch(0, 1, hw, W), ch(1, 1, hw, W))
    KV = _rr([(0,) + i for i in t0], [(1,) + i for i in t1])

    wo_bounds = []
    r = 0
    for n in (512,) * 7 + (256, 128, 128):
        wo_bounds.append((r, n))
        r += n
    assert r == H * DH
    NWO = len(wo_bounds)

    def kernel(x_hbm, k_hbm, v_hbm, wq_hbm, wo_hbm, w3_hbm, w4_hbm, o_ref,
               x_v, wq_v, wo_v, w3_v, w4_v, kv, q_v, o_v, sems, gsems, wosems):
        def start(src, dst, sem, pr):
            pltpu.make_async_copy(src, dst, sem).start(priority=pr)

        def wait(ref, sem):
            pltpu.make_async_copy(ref, ref, sem).wait()

        def issue_kv(g):
            for (pr, which, hoff, r, n) in KV:
                src = (k_hbm, v_hbm)[which]
                start(src.at[0, g * HPG + hoff, pl.ds(SK - W + r, n), :],
                      kv.at[g, which * HPG + hoff, pl.ds(r, n), :], gsems.at[g], pr)

        def issue_rows(src, dst, r0, r1, rows, sem):
            sp = _spans(r0, r1, rows)
            half = (len(sp) + 1) // 2
            for pr, (r, n) in _rr([(0, s) for s in sp[:half]], [(1, s) for s in sp[half:]]):
                start(src.at[pl.ds(r, n), :], dst.at[pl.ds(r, n), :], sem, pr)

        def issue_wq():
            cw = H * DH // 2
            a = [(0, (r, cc)) for r in range(0, D // 2, 8) for cc in (0, cw)]
            b = [(1, (r, cc)) for r in range(D // 2, D, 8) for cc in (0, cw)]
            for pr, (r, cc) in _rr(a, b):
                start(wq_hbm.at[pl.ds(r, 8), pl.ds(cc, cw)],
                      wq_v.at[pl.ds(r, 8), pl.ds(cc, cw)], sems.at[1], pr)

        start(x_hbm, x_v, sems.at[0], 0)
        issue_wq()
        for g in range(LOOK):
            issue_kv(g)
        wait(x_v, sems.at[0])
        x = x_v[0].astype(f32)
        xn = _ln(x)
        xn8 = jnp.broadcast_to(xn, (8, D)).astype(bf16)
        wait(wq_v, sems.at[1])
        q = jnp.dot(xn8, wq_v[...], preferred_element_type=f32) * (DH ** -0.5)
        q_v[...] = q.astype(bf16)

        def issue_tail(i):
            if i == 0:
                issue_rows(w3_hbm, w3_v, 0, F, 32, sems.at[2])
                issue_rows(w4_hbm, w4_v, 0, F, 32, sems.at[3])
            if i == LOOK - 1:
                for j, (r, n) in enumerate(wo_bounds):
                    issue_rows(wo_hbm, wo_v, r, r + n, 32, wosems.at[j])

        def compute(g):
            for hoff in range(HPG):
                h = g * HPG + hoff
                col = h * DH if isinstance(h, int) else pl.multiple_of(h * DH, DH)
                qh = q_v[:, pl.ds(col, DH)]
                s = jax.lax.dot_general(qh, kv[g, hoff], (((1,), (1,)), ((), ())),
                                        preferred_element_type=f32)
                m = jnp.max(s, axis=-1, keepdims=True)
                p = jnp.exp(s - m)
                l = jnp.sum(p, axis=-1, keepdims=True)
                o = jnp.dot(p.astype(bf16), kv[g, HPG + hoff],
                            preferred_element_type=f32) / l
                o_v[:, pl.ds(col, DH)] = o.astype(bf16)

        def body(g, carry):
            wait(kv.at[g], gsems.at[g])
            issue_kv(g + LOOK)
            compute(g)
            return carry

        jax.lax.fori_loop(0, NG - LOOK, body, 0)
        for i in range(LOOK):
            g = NG - LOOK + i
            wait(kv.at[g], gsems.at[g])
            issue_tail(i)
            compute(g)
        wait(w3_v, sems.at[2])
        wait(w4_v, sems.at[3])
        ln2 = _ln(xn)
        ln8 = jnp.broadcast_to(ln2, (8, D)).astype(bf16)
        h1 = jax.nn.gelu(
            jax.lax.dot_general(ln8, w3_v[...], (((1,), (1,)), ((), ())),
                                preferred_element_type=f32), approximate=True)
        h2 = jnp.dot(h1.astype(bf16), w4_v[...], preferred_element_type=f32)
        gate = jax.nn.silu(xn + h2[0:1])
        acc = jnp.zeros((8, D), f32)
        for j, (r, n) in enumerate(wo_bounds):
            wait(wo_v.at[pl.ds(r, n), :], wosems.at[j])
            acc = acc + jnp.dot(o_v[:, r:r + n], wo_v[r:r + n, :], preferred_element_type=f32)
        o_ref[0] = (x + acc[0:1] * gate).astype(o_ref.dtype)

    return pl.pallas_call(
        kernel,
        in_specs=[pl.BlockSpec(memory_space=pl.ANY)] * 7,
        out_specs=pl.BlockSpec(memory_space=pltpu.VMEM),
        out_shape=jax.ShapeDtypeStruct((1, 1, D), bf16),
        scratch_shapes=[
            pltpu.VMEM((1, 1, D), bf16), pltpu.VMEM((D, H * DH), bf16), pltpu.VMEM((H * DH, D), bf16),
            pltpu.VMEM((F, D), bf16), pltpu.VMEM((F, D), bf16),
            pltpu.VMEM((NG, 2 * HPG, W, DH), bf16),
            pltpu.VMEM((8, H * DH), bf16), pltpu.VMEM((8, H * DH), bf16),
            pltpu.SemaphoreType.DMA((4,)), pltpu.SemaphoreType.DMA((NG,)),
            pltpu.SemaphoreType.DMA((NWO,))],
        compiler_params=pltpu.CompilerParams(vmem_limit_bytes=110 * 1024 * 1024),
    )(A_x, A_k_cache, A_v_cache, A_wq, A_wo, B_w3.T, B_w4)
```

```python
import jax
import jax.numpy as jnp
import jax.experimental.pallas as pl
import jax.experimental.pallas.tpu as pltpu

f32, bf16 = jnp.float32, jnp.bfloat16


def _ln(x, eps=1e-5):
    m = jnp.mean(x, axis=-1, keepdims=True)
    xc = x - m
    v = jnp.mean(xc * xc, axis=-1, keepdims=True)
    return xc * jax.lax.rsqrt(v + eps)


@jax.jit
def pallas_recurrent_scan__sliding_block_cached__mixer_s_mlp__decode_kernel(
    A_x: jax.Array,
    A_k_cache: jax.Array,
    A_v_cache: jax.Array,
    A_wq: jax.Array,
    A_wo: jax.Array,
    B_x: jax.Array,
    B_w1: jax.Array,
    B_w2: jax.Array,
    B_w3: jax.Array,
    B_w4: jax.Array,
):
    _, _, D = A_x.shape
    _, H, SK, DH = A_k_cache.shape
    F = B_w3.shape[1]
    W = min(4096, max(256, SK // 4))
    HPG = 2
    NG = H // HPG
    C = 128
    hw = W // 2
    NR = hw // C
    RPU = NR // HPG
    LOOKU = HPG + 2
    MLP_AT = 2
    wo_groups = (512,) * 7 + (256, 256)
    assert sum(wo_groups) == H * DH
    NWO = len(wo_groups)
    wo_off = [sum(wo_groups[:j]) for j in range(NWO)]
    n_first = max(j for j in range(NWO + 1) if sum(wo_groups[:j]) <= H * DH // 2)
    streams = [(w, h) for w in (0, 1) for h in range(HPG)]

    def kernel(x_hbm, k_hbm, v_hbm, wq_hbm, wo_hbm, w3_hbm, w4_hbm, o_ref,
               x_v, wq_v, wo_v, w3_v, w4_v, kv, xn_v, o_v, gate_v):
        def inner(sems, gsems, wosems):
            def start(src, dst, sem, pr):
                pltpu.make_async_copy(src, dst, sem).start(priority=pr)

            def wait(ref, sem):
                pltpu.make_async_copy(ref, ref, sem).wait()

            def loop(lo, hi, body):
                def b(i, c):
                    body(i)
                    return c
                jax.lax.fori_loop(lo, hi, b, 0)

            def issue_unit(u):
                g = u // HPG
                j0 = (u % HPG) * RPU

                def rnd(j):
                    for (which, hoff) in streams:
                        for pr in (0, 1):
                            r = pl.multiple_of((j0 + j) * C + pr * hw, C)
                            src = (k_hbm, v_hbm)[which]
                            start(src.at[0, g * HPG + hoff, pl.ds(SK - W + r, C), :],
                                  kv.at[g, which * HPG + hoff, pl.ds(r, C), :], gsems.at[g], pr)
                loop(0, RPU, rnd)

            def issue_rows(src, dst, r0, nrows, sem, rows=32):
                n = nrows // rows
                assert n * rows == nrows
                half = (n + 1) // 2

                def it(i):
                    ra = pl.multiple_of(r0 + i * rows, rows)
                    rb = pl.multiple_of(r0 + (i + half) * rows, rows)
                    start(src.at[pl.ds(ra, rows), :], dst.at[pl.ds(ra, rows), :], sem, 0)
                    start(src.at[pl.ds(rb, rows), :], dst.at[pl.ds(rb, rows), :], sem, 1)
                loop(0, n // 2, it)
                if n % 2:
                    i = half - 1
                    start(src.at[pl.ds(r0 + i * rows, rows), :], dst.at[pl.ds(r0 + i * rows, rows), :], sem, 0)

            def issue_wq():
                cw = H * DH // 2

                def it(i):
                    for cc in (0, cw):
                        for pr in (0, 1):
                            r = pl.multiple_of(i * 8 + pr * (D // 2), 8)
                            start(wq_hbm.at[pl.ds(r, 8), pl.ds(cc, cw)],
                                  wq_v.at[pl.ds(r, 8), pl.ds(cc, cw)], sems.at[1], pr)
                loop(0, D // 16, it)

            def issue_wo(js):
                for j in js:
                    issue_rows(wo_hbm, wo_v, wo_off[j], wo_groups[j], wosems.at[j])

            start(x_hbm, x_v, sems.at[0], 0)
            issue_wq()
            issue_rows(w3_hbm, w3_v, 0, F, sems.at[2])
            issue_rows(w4_hbm, w4_v, 0, F, sems.at[3])
            loop(0, MLP_AT, issue_unit)
            wait(x_v, sems.at[0])
            x = x_v[0].astype(f32)
            xn = _ln(x)
            xn_v[...] = jnp.broadcast_to(xn, (8, D)).astype(bf16)
            wait(w3_v, sems.at[2])
            wait(w4_v, sems.at[3])
            ln2 = _ln(xn)
            ln8 = jnp.broadcast_to(ln2, (8, D)).astype(bf16)
            h1 = jax.nn.gelu(
                jax.lax.dot_general(ln8, w3_v[...], (((1,), (1,)), ((), ())),
                                    preferred_element_type=f32), approximate=True)
            h2 = jnp.dot(h1.astype(bf16), w4_v[...], preferred_element_type=f32)
            gate_v[...] = jax.nn.silu(xn + h2[0:1])
            wait(wq_v, sems.at[1])
            loop(MLP_AT, LOOKU, issue_unit)

            def head(hh):
                g = hh // HPG
                hoff = hh % HPG

                @pl.when(hoff == 0)
                def _():
                    wait(kv.at[g], gsems.at[g])

                col = pl.multiple_of(hh * DH, DH)
                qh = (jnp.dot(xn_v[...], wq_v[:, pl.ds(col, DH)], preferred_element_type=f32)
                      * (DH ** -0.5)).astype(bf16)
                s = jax.lax.dot_general(qh, kv[g, hoff], (((1,), (1,)), ((), ())),
                                        preferred_element_type=f32)
                m = jnp.max(s, axis=-1, keepdims=True)
                p = jnp.exp(s - m)
                l = jnp.sum(p, axis=-1, keepdims=True)
                o = jnp.dot(p.astype(bf16), kv[g, HPG + hoff],
                            preferred_element_type=f32) / l
                o_v[:, pl.ds(col, DH)] = o.astype(bf16)

                @pl.when(hh + LOOKU < H)
                def _():
                    issue_unit(hh + LOOKU)

                @pl.when(hh + LOOKU == H)
                def _():
                    issue_wo(range(n_first))

                @pl.when(hh + LOOKU == H + 1)
                def _():
                    issue_wo(range(n_first, NWO))
            loop(0, H, head)

            acc = jnp.zeros((8, D), f32)
            j = 0
            while j < NWO:
                k = j
                while k < NWO and wo_groups[k] == wo_groups[j]:
                    k += 1
                n = wo_groups[j]

                def wo_step(i, acc, j=j, n=n):
                    r = pl.multiple_of(wo_off[j] + i * n, n)
                    wait(wo_v.at[pl.ds(r, n), :], wosems.at[j + i])
                    return acc + jnp.dot(o_v[:, pl.ds(r, n)], wo_v[pl.ds(r, n), :],
                                         preferred_element_type=f32)
                acc = jax.lax.fori_loop(0, k - j, wo_step, acc)
                j = k
            o_ref[0] = (x + acc[0:1] * gate_v[...]).astype(o_ref.dtype)

        pl.run_scoped(inner, pltpu.SemaphoreType.DMA((4,)), pltpu.SemaphoreType.DMA((NG,)),
                      pltpu.SemaphoreType.DMA((NWO,)))

    return pl.pallas_call(
        kernel,
        in_specs=[pl.BlockSpec(memory_space=pl.ANY)] * 7,
        out_specs=pl.BlockSpec(memory_space=pltpu.VMEM),
        out_shape=jax.ShapeDtypeStruct((1, 1, D), bf16),
        scratch_shapes=[
            pltpu.VMEM((1, 1, D), bf16), pltpu.VMEM((D, H * DH), bf16), pltpu.VMEM((H * DH, D), bf16),
            pltpu.VMEM((F, D), bf16), pltpu.VMEM((F, D), bf16),
            pltpu.VMEM((NG, 2 * HPG, W, DH), bf16),
            pltpu.VMEM((8, D), bf16), pltpu.VMEM((8, H * DH), bf16), pltpu.VMEM((1, D), f32)],
        compiler_params=pltpu.CompilerParams(vmem_limit_bytes=110 * 1024 * 1024),
    )(A_x, A_k_cache, A_v_cache, A_wq, A_wo, B_w3.T, B_w4)
```

```python
import jax
import jax.numpy as jnp
import jax.experimental.pallas as pl
import jax.experimental.pallas.tpu as pltpu

f32, bf16 = jnp.float32, jnp.bfloat16


def _ln(x, eps=1e-5):
    m = jnp.mean(x, axis=-1, keepdims=True)
    xc = x - m
    v = jnp.mean(xc * xc, axis=-1, keepdims=True)
    return xc * jax.lax.rsqrt(v + eps)


@jax.jit
def pallas_recurrent_scan__sliding_block_cached__mixer_s_mlp__decode_kernel(
    A_x: jax.Array,
    A_k_cache: jax.Array,
    A_v_cache: jax.Array,
    A_wq: jax.Array,
    A_wo: jax.Array,
    B_x: jax.Array,
    B_w1: jax.Array,
    B_w2: jax.Array,
    B_w3: jax.Array,
    B_w4: jax.Array,
):
    _, _, D = A_x.shape
    _, H, SK, DH = A_k_cache.shape
    F = B_w3.shape[1]
    W = min(4096, max(256, SK // 4))
    C = 128
    HPG = 4
    NG = H // HPG
    PART = W // 2
    NJ = PART // C
    NMIX = (NG - 1) * 2 * NJ
    NKV = NG * 2 * NJ
    WR = 32
    WO_ROWS = 512
    NWO = H * DH // WO_ROWS
    RPG = WO_ROWS // 256
    NWR = NWO * RPG
    TOT = NKV + NWR
    T1 = (NG - 2) * HPG
    T2 = NG * HPG
    NSTEP = T2 + HPG
    EXTRA = 12
    INC = 4
    MLP_AT = 24
    LOOK = 2 * NJ + EXTRA
    assert HPG == 4 and NJ == 16 and RPG == 2 and H * DH % WO_ROWS == 0
    tail_cum = [min(TOT, NKV + EXTRA + -(-(TOT - NKV - EXTRA) * (t - T2 + 1) // HPG))
                for t in range(T2, NSTEP)]
    assert tail_cum[-1] == TOT

    srl = jax.lax.shift_right_logical

    def kernel(x_hbm, k_hbm, v_hbm, wq_hbm, wo_hbm, w3_hbm, w4_hbm, o_ref,
               x_v, wq_v, wo_v, w3_v, w4_v, kv, xn_v, o_v, gate_v, p_v, l_v):
        def inner(sems, gsems, wosems):
            def start(src, dst, sem, pr):
                pltpu.make_async_copy(src, dst, sem).start(priority=pr)

            def wait(ref, sem):
                pltpu.make_async_copy(ref, ref, sem).wait()

            def loop(lo, hi, body):
                def b(i, c):
                    body(i)
                    return c
                jax.lax.fori_loop(lo, hi, b, 0)

            def kv_half(R):
                mixed = R < NMIX
                g = jnp.minimum(srl(R, 5), NG - 1)
                j = jnp.where(mixed, srl(R & 31, 1), R & 15)
                w = jnp.where(mixed, R & 1, srl(R - NMIX, 4) & 1)
                si = jnp.where(mixed, g, NG - 1 + w)
                h0 = g * HPG

                def go(src, wi):
                    for h in range(HPG):
                        for s in range(2):
                            r = pl.multiple_of(s * PART + j * C, C)
                            start(src.at[0, h0 + h, pl.ds(SK - W + r, C), :],
                                  kv.at[g, wi * HPG + h, pl.ds(r, C), :], gsems.at[si], s)

                @pl.when(w == 0)
                def _():
                    go(k_hbm, 0)

                @pl.when(w == 1)
                def _():
                    go(v_hbm, 1)

            def wo_round(r):
                gi = srl(r, 1)
                base = gi * WO_ROWS + (r & 1) * 128
                for i in range(4):
                    for pr in (0, 1):
                        row = pl.multiple_of(base + i * WR + pr * (WO_ROWS // 2), WR)
                        start(wo_hbm.at[pl.ds(row, WR), :], wo_v.at[pl.ds(row, WR), :],
                              wosems.at[gi], pr)

            def issue_rows(src, dst, nrows, sem):
                n = nrows // WR
                assert n * WR == nrows
                half = (n + 1) // 2

                def it(i):
                    ra = pl.multiple_of(i * WR, WR)
                    rb = pl.multiple_of((i + half) * WR, WR)
                    start(src.at[pl.ds(ra, WR), :], dst.at[pl.ds(ra, WR), :], sem, 0)
                    start(src.at[pl.ds(rb, WR), :], dst.at[pl.ds(rb, WR), :], sem, 1)
                loop(0, n // 2, it)
                if n % 2:
                    r = (half - 1) * WR
                    start(src.at[pl.ds(r, WR), :], dst.at[pl.ds(r, WR), :], sem, 0)

            def issue_wq():
                cw = H * DH // 2

                def it(i):
                    for cc in (0, cw):
                        for pr in (0, 1):
                            r = pl.multiple_of(i * 8 + pr * (D // 2), 8)
                            start(wq_hbm.at[pl.ds(r, 8), pl.ds(cc, cw)],
                                  wq_v.at[pl.ds(r, 8), pl.ds(cc, cw)], sems.at[1], pr)
                loop(0, D // 16, it)

            start(x_hbm, x_v, sems.at[0], 0)
            issue_wq()
            issue_rows(w3_hbm, w3_v, F, sems.at[2])
            issue_rows(w4_hbm, w4_v, F, sems.at[3])
            loop(0, MLP_AT, kv_half)

            wait(x_v, sems.at[0])
            x = x_v[0].astype(f32)
            xn = _ln(x)
            xn_v[...] = jnp.broadcast_to(xn, (8, D)).astype(bf16)
            wait(w3_v, sems.at[2])
            wait(w4_v, sems.at[3])
            ln8 = jnp.broadcast_to(_ln(xn), (8, D)).astype(bf16)
            h1 = jax.nn.gelu(
                jax.lax.dot_general(ln8, w3_v[...], (((1,), (1,)), ((), ())),
                                    preferred_element_type=f32), approximate=True)
            h2 = jnp.dot(h1.astype(bf16), w4_v[...], preferred_element_type=f32)
            gate_v[...] = jax.nn.silu(xn + h2[0:1])
            wait(wq_v, sems.at[1])
            loop(MLP_AT, LOOK, kv_half)

            def cum(t):
                g = srl(t, 2)
                i = t & 3
                a = 2 * NJ * (g + 1) + EXTRA + jnp.where(i == HPG - 1, 2 * NJ, INC * (i + 1))
                b = NMIX + EXTRA + (t - T1 + 1) * ((NKV - NMIX) // (2 * HPG))
                out = jnp.where(t < T1, a, b)
                for k, tt in enumerate(range(T2, NSTEP)):
                    out = jnp.where(t == tt, tail_cum[k], out)
                return out

            def step(t, prev):
                pv_only = t >= T2
                qk_only = jnp.logical_and(t >= T2 - HPG, t < T2)
                hh = jnp.where(pv_only, t - HPG, t)
                i = t & 3
                g = srl(hh, 2)
                col = pl.multiple_of(hh * DH, DH)

                @pl.when(jnp.logical_and(i == 0, t < T2 - HPG))
                def _():
                    wait(kv.at[g], gsems.at[g])

                @pl.when(t == T2 - HPG)
                def _():
                    wait(kv.at[NG - 1, pl.ds(0, HPG)], gsems.at[NG - 1])

                @pl.when(t == T2)
                def _():
                    wait(kv.at[NG - 1, pl.ds(HPG, HPG)], gsems.at[NG])

                @pl.when(t < T2)
                def _():
                    q = (jnp.dot(xn_v[...], wq_v[:, pl.ds(col, DH)], preferred_element_type=f32)
                         * (DH ** -0.5)).astype(bf16)
                    s = jax.lax.dot_general(q, kv[g, i], (((1,), (1,)), ((), ())),
                                            preferred_element_type=f32)
                    p = jnp.exp(s - jnp.max(s, axis=-1, keepdims=True))
                    l_v[i] = jnp.broadcast_to(jnp.sum(p, axis=-1, keepdims=True), (8, DH))
                    p_v[i] = p.astype(bf16)

                @pl.when(jnp.logical_not(qk_only))
                def _():
                    o = jnp.dot(p_v[i], kv[g, HPG + i], preferred_element_type=f32) / l_v[i]
                    o_v[:, pl.ds(col, DH)] = o.astype(bf16)

                hi = cum(t)
                loop(prev, jnp.minimum(hi, NKV), kv_half)
                loop(jnp.maximum(prev, NKV) - NKV, hi - NKV, wo_round)
                return hi
            jax.lax.fori_loop(0, NSTEP, step, jnp.int32(LOOK))

            def wo_step(i, acc):
                r = pl.multiple_of(i * WO_ROWS, WO_ROWS)
                wait(wo_v.at[pl.ds(r, WO_ROWS), :], wosems.at[i])
                return acc + jnp.dot(o_v[:, pl.ds(r, WO_ROWS)], wo_v[pl.ds(r, WO_ROWS), :],
                                     preferred_element_type=f32)
            acc = jax.lax.fori_loop(0, NWO, wo_step, jnp.zeros((8, D), f32))
            o_ref[0] = (x + acc[0:1] * gate_v[...]).astype(o_ref.dtype)

        pl.run_scoped(inner, pltpu.SemaphoreType.DMA((4,)), pltpu.SemaphoreType.DMA((NG + 1,)),
                      pltpu.SemaphoreType.DMA((NWO,)))

    return pl.pallas_call(
        kernel,
        in_specs=[pl.BlockSpec(memory_space=pl.ANY)] * 7,
        out_specs=pl.BlockSpec(memory_space=pltpu.VMEM),
        out_shape=jax.ShapeDtypeStruct((1, 1, D), bf16),
        scratch_shapes=[
            pltpu.VMEM((1, 1, D), bf16), pltpu.VMEM((D, H * DH), bf16), pltpu.VMEM((H * DH, D), bf16),
            pltpu.VMEM((F, D), bf16), pltpu.VMEM((F, D), bf16),
            pltpu.VMEM((NG, 2 * HPG, W, DH), bf16),
            pltpu.VMEM((8, D), bf16), pltpu.VMEM((8, H * DH), bf16), pltpu.VMEM((1, D), f32),
            pltpu.VMEM((HPG, 8, W), bf16), pltpu.VMEM((HPG, 8, DH), f32)],
        compiler_params=pltpu.CompilerParams(vmem_limit_bytes=110 * 1024 * 1024),
    )(A_x, A_k_cache, A_v_cache, A_wq, A_wo, B_w3.T, B_w4)
```

```python
import jax
import jax.numpy as jnp
import jax.experimental.pallas as pl
import jax.experimental.pallas.tpu as pltpu

f32, bf16 = jnp.float32, jnp.bfloat16


def _ln(x, eps=1e-5):
    m = jnp.mean(x, axis=-1, keepdims=True)
    xc = x - m
    v = jnp.mean(xc * xc, axis=-1, keepdims=True)
    return xc * jax.lax.rsqrt(v + eps)


@jax.jit
def pallas_recurrent_scan__sliding_block_cached__mixer_s_mlp__decode_kernel(
    A_x: jax.Array,
    A_k_cache: jax.Array,
    A_v_cache: jax.Array,
    A_wq: jax.Array,
    A_wo: jax.Array,
    B_x: jax.Array,
    B_w1: jax.Array,
    B_w2: jax.Array,
    B_w3: jax.Array,
    B_w4: jax.Array,
):
    _, _, D = A_x.shape
    _, H, SK, DH = A_k_cache.shape
    F = B_w3.shape[1]
    W = min(4096, max(256, SK // 4))
    C = 128
    HPG = 4
    NG = H // HPG
    PART = W // 2
    NJ = PART // C
    NMIX = (NG - 1) * 2 * NJ
    NKV = NG * 2 * NJ
    WR = 32
    wo_plan = [(512, 8)] * 7 + [(256, 4), (128, 2), (64, 0), (64, 0)]
    N_MXU = 7
    WO_ROWS = 512
    wo_groups = [n for n, _ in wo_plan]
    assert sum(wo_groups) == H * DH and all(n == WO_ROWS for n in wo_groups[:N_MXU])
    NWO = len(wo_groups)
    wo_off = [sum(wo_groups[:j]) for j in range(NWO)]
    wo_desc = []
    for gi, (n, n0) in enumerate(wo_plan):
        rows = [wo_off[gi] + k * WR for k in range(n // WR)]
        a, b = rows[:n0], rows[n0:]
        ia = ib = 0
        while ia < len(a) or ib < len(b):
            if ib >= len(b) or (ia < len(a) and ia * len(b) <= ib * len(a)):
                wo_desc.append((a[ia], 0, gi))
                ia += 1
            else:
                wo_desc.append((b[ib], 1, gi))
                ib += 1
    wo_steps = (32, 32, 32, 8, 8, 8, 8)
    assert sum(wo_steps) == len(wo_desc)
    R_V = wo_off[N_MXU]
    N_V = H * DH - R_V
    T1 = (NG - 2) * HPG
    T2 = NG * HPG
    NSTEP = T2 + HPG
    EXTRA = 12
    INC = 4
    MLP_AT = 24
    LOOK = 2 * NJ + EXTRA
    FIRST_WO_STEP = NSTEP - len(wo_steps)
    assert HPG == 4 and NJ == 16 and DH == 128 and N_V % DH == 0

    srl = jax.lax.shift_right_logical

    def kernel(x_hbm, k_hbm, v_hbm, wq_hbm, wo_hbm, w3_hbm, w4_hbm, o_ref,
               x_v, wq_v, wo_v, w3_v, w4_v, kv, xn_v, o_v, gate_v, p_v, l_v, obc_v):
        def inner(sems, gsems, wosems):
            def start(src, dst, sem, pr):
                pltpu.make_async_copy(src, dst, sem).start(priority=pr)

            def wait(ref, sem):
                pltpu.make_async_copy(ref, ref, sem).wait()

            def loop(lo, hi, body):
                def b(i, c):
                    body(i)
                    return c
                jax.lax.fori_loop(lo, hi, b, 0)

            def kv_half(R):
                mixed = R < NMIX
                g = jnp.minimum(srl(R, 5), NG - 1)
                j = jnp.where(mixed, srl(R & 31, 1), R & 15)
                w = jnp.where(mixed, R & 1, srl(R - NMIX, 4) & 1)
                si = jnp.where(mixed, g, NG - 1 + w)
                h0 = g * HPG

                def go(src, wi):
                    for h in range(HPG):
                        for s in range(2):
                            r = pl.multiple_of(s * PART + j * C, C)
                            start(src.at[0, h0 + h, pl.ds(SK - W + r, C), :],
                                  kv.at[g, wi * HPG + h, pl.ds(r, C), :], gsems.at[si], s)

                @pl.when(w == 0)
                def _():
                    go(k_hbm, 0)

                @pl.when(w == 1)
                def _():
                    go(v_hbm, 1)

            def wo_issue(k):
                lo = sum(wo_steps[:k])
                for (row, pr, gi) in wo_desc[lo:lo + wo_steps[k]]:
                    start(wo_hbm.at[pl.ds(row, WR), :], wo_v.at[pl.ds(row, WR), :],
                          wosems.at[gi], pr)

            def issue_rows(src, dst, nrows, sem):
                n = nrows // WR
                assert n * WR == nrows
                half = (n + 1) // 2

                def it(i):
                    ra = pl.multiple_of(i * WR, WR)
                    rb = pl.multiple_of((i + half) * WR, WR)
                    start(src.at[pl.ds(ra, WR), :], dst.at[pl.ds(ra, WR), :], sem, 0)
                    start(src.at[pl.ds(rb, WR), :], dst.at[pl.ds(rb, WR), :], sem, 1)
                loop(0, n // 2, it)
                if n % 2:
                    r = (half - 1) * WR
                    start(src.at[pl.ds(r, WR), :], dst.at[pl.ds(r, WR), :], sem, 0)

            def issue_wq():
                cw = H * DH // 2

                def it(i):
                    for cc in (0, cw):
                        for pr in (0, 1):
                            r = pl.multiple_of(i * 8 + pr * (D // 2), 8)
                            start(wq_hbm.at[pl.ds(r, 8), pl.ds(cc, cw)],
                                  wq_v.at[pl.ds(r, 8), pl.ds(cc, cw)], sems.at[1], pr)
                loop(0, D // 16, it)

            start(x_hbm, x_v, sems.at[0], 0)
            issue_wq()
            issue_rows(w3_hbm, w3_v, F, sems.at[2])
            issue_rows(w4_hbm, w4_v, F, sems.at[3])
            loop(0, MLP_AT, kv_half)

            wait(x_v, sems.at[0])
            x = x_v[0].astype(f32)
            xn = _ln(x)
            xn_v[...] = jnp.broadcast_to(xn, (8, D)).astype(bf16)
            wait(w3_v, sems.at[2])
            wait(w4_v, sems.at[3])
            ln8 = jnp.broadcast_to(_ln(xn), (8, D)).astype(bf16)
            h1 = jax.nn.gelu(
                jax.lax.dot_general(ln8, w3_v[...], (((1,), (1,)), ((), ())),
                                    preferred_element_type=f32), approximate=True)
            h2 = jnp.dot(h1.astype(bf16), w4_v[...], preferred_element_type=f32)
            gate_v[...] = jax.nn.silu(xn + h2[0:1])
            wait(wq_v, sems.at[1])
            loop(MLP_AT, LOOK, kv_half)

            def cum(t):
                g = srl(t, 2)
                i = t & 3
                a = 2 * NJ * (g + 1) + EXTRA + jnp.where(i == HPG - 1, 2 * NJ, INC * (i + 1))
                b = NMIX + EXTRA + (t - T1 + 1) * ((NKV - NMIX) // (2 * HPG))
                return jnp.minimum(jnp.where(t < T1, a, b), NKV)

            def step(t, prev):
                pv_only = t >= T2
                qk_only = jnp.logical_and(t >= T2 - HPG, t < T2)
                hh = jnp.where(pv_only, t - HPG, t)
                i = t & 3
                g = srl(hh, 2)
                col = pl.multiple_of(hh * DH, DH)

                @pl.when(jnp.logical_and(i == 0, t < T2 - HPG))
                def _():
                    wait(kv.at[g], gsems.at[g])

                @pl.when(t == T2 - HPG)
                def _():
                    wait(kv.at[NG - 1, pl.ds(0, HPG)], gsems.at[NG - 1])

                @pl.when(t == T2)
                def _():
                    wait(kv.at[NG - 1, pl.ds(HPG, HPG)], gsems.at[NG])

                @pl.when(t < T2)
                def _():
                    q = jnp.dot(xn_v[...], wq_v[:, pl.ds(col, DH)],
                                preferred_element_type=f32).astype(bf16)
                    s = jax.lax.dot_general(q, kv[g, i], (((1,), (1,)), ((), ())),
                                            preferred_element_type=f32) * (DH ** -0.5)
                    p = jnp.exp(s - jnp.max(s, axis=-1, keepdims=True))
                    l_v[i] = jnp.broadcast_to(jnp.sum(p, axis=-1, keepdims=True), (8, DH))
                    p_v[i] = p.astype(bf16)

                @pl.when(jnp.logical_not(qk_only))
                def _():
                    o = jnp.dot(p_v[i], kv[g, HPG + i], preferred_element_type=f32) / l_v[i]
                    o_v[:, pl.ds(col, DH)] = o.astype(bf16)

                hi = cum(t)
                loop(prev, hi, kv_half)
                for k in range(len(wo_steps)):
                    @pl.when(t == FIRST_WO_STEP + k)
                    def _(k=k):
                        wo_issue(k)
                return hi
            jax.lax.fori_loop(0, NSTEP, step, jnp.int32(LOOK))

            eye = (jax.lax.broadcasted_iota(jnp.int32, (DH, DH), 0)
                   == jax.lax.broadcasted_iota(jnp.int32, (DH, DH), 1))
            for b in range(N_V // DH):
                ob = o_v[0:1, R_V + b * DH:R_V + (b + 1) * DH].astype(f32)
                diag = jnp.where(eye, jnp.broadcast_to(ob, (DH, DH)), 0.0).astype(bf16)
                obc_v[b * DH:(b + 1) * DH, :] = jnp.dot(
                    diag, jnp.ones((DH, DH), bf16), preferred_element_type=f32)

            def wo_step(i, acc):
                r = pl.multiple_of(i * WO_ROWS, WO_ROWS)
                wait(wo_v.at[pl.ds(r, WO_ROWS), :], wosems.at[i])
                return acc + jnp.dot(o_v[:, pl.ds(r, WO_ROWS)], wo_v[pl.ds(r, WO_ROWS), :],
                                     preferred_element_type=f32)
            acc = jax.lax.fori_loop(0, N_MXU, wo_step, jnp.zeros((8, D), f32))
            gate = gate_v[...]
            base = x + acc[0:1] * gate
            psum = [jnp.zeros((8, DH), f32) for _ in range(D // DH)]
            for gi in range(N_MXU, NWO):
                r0, n = wo_off[gi], wo_groups[gi]
                wait(wo_v.at[pl.ds(r0, n), :], wosems.at[gi])
                for rr in range(r0, r0 + n, 8):
                    ob = obc_v[rr - R_V:rr - R_V + 8, :]
                    for jj in range(D // DH):
                        psum[jj] = psum[jj] + (
                            wo_v[rr:rr + 8, jj * DH:(jj + 1) * DH].astype(f32) * ob)
            sv = jnp.concatenate([jnp.sum(p, axis=0, keepdims=True) for p in psum], axis=1)
            o_ref[0] = (base + sv * gate).astype(o_ref.dtype)

        pl.run_scoped(inner, pltpu.SemaphoreType.DMA((4,)), pltpu.SemaphoreType.DMA((NG + 1,)),
                      pltpu.SemaphoreType.DMA((NWO,)))

    return pl.pallas_call(
        kernel,
        in_specs=[pl.BlockSpec(memory_space=pl.ANY)] * 7,
        out_specs=pl.BlockSpec(memory_space=pltpu.VMEM),
        out_shape=jax.ShapeDtypeStruct((1, 1, D), bf16),
        scratch_shapes=[
            pltpu.VMEM((1, 1, D), bf16), pltpu.VMEM((D, H * DH), bf16), pltpu.VMEM((H * DH, D), bf16),
            pltpu.VMEM((F, D), bf16), pltpu.VMEM((F, D), bf16),
            pltpu.VMEM((NG, 2 * HPG, W, DH), bf16),
            pltpu.VMEM((8, D), bf16), pltpu.VMEM((8, H * DH), bf16), pltpu.VMEM((1, D), f32),
            pltpu.VMEM((HPG, 8, W), bf16), pltpu.VMEM((HPG, 8, DH), f32),
            pltpu.VMEM((N_V, DH), f32)],
        compiler_params=pltpu.CompilerParams(vmem_limit_bytes=110 * 1024 * 1024),
    )(A_x, A_k_cache, A_v_cache, A_wq, A_wo, B_w3.T, B_w4)
```
